```python
import os as _os
_os.environ.setdefault("JAX_PLATFORMS", "cpu")
import jax
import jax.numpy as jnp

def _softmax(x, axis=-1):
    return jax.nn.softmax(x, axis=axis)
def _gelu(x):
    return jax.nn.gelu(x, approximate=True)
def _silu(x):
    return jax.nn.silu(x)
def _sigmoid(x):
    return jax.nn.sigmoid(x)
def _layernorm(x, axis=-1, eps=1e-5):
    m = jnp.mean(x, axis=axis, keepdims=True)
    v = jnp.var(x, axis=axis, keepdims=True)
    return (x - m) / jnp.sqrt(v + eps)
def _scatter_add(tgt, idx, src, axis=0):
    return tgt.at[idx].add(src)
def _segment_sum(src, seg, n):
    return jax.ops.segment_sum(src, seg, n)
class _Rng:
    def __init__(self, key):
        self._k = key
    def _next(self):
        self._k, sub = jax.random.split(self._k)
        return sub
    def normal(self, shape):
        return jax.random.normal(self._next(), shape, dtype=jnp.bfloat16)
    def randint(self, lo, hi, shape):
        return jax.random.randint(self._next(), shape, lo, hi, dtype=jnp.int32)
    def uniform(self, shape, lo=0.0, hi=1.0):
        return jax.random.uniform(self._next(), shape, jnp.bfloat16, lo, hi)
    def permutation(self, n):
        return jax.random.permutation(self._next(), n)


kernel_name = 'standalone__se_block__vision'

def setup_inputs():
    _rng = _Rng(jax.random.key(int.from_bytes(__import__("os").urandom(4), "little")))
    _w = (lambda a: (lambda t: t.astype(jnp.bfloat16) if jnp.issubdtype(t.dtype, jnp.floating) else t)(jnp.asarray(a)))
    H = W = 384
    C = 192; r = max(C // 16, 4)
    return {
        "x": _w((lambda *s: _rng.normal(s) * 0.8)(1, H, W, C)),
        "w_down": _w((lambda *s: _rng.normal(s) * 0.8)(C, r)),
        "w_up": _w((lambda *s: _rng.normal(s) * 0.8)(r, C)),
    }

def reference(x, w_down, w_up):
    s = x.mean(axis=(1, 2))
    s = _sigmoid(_silu(s @ w_down) @ w_up)
    return x * s[:, None, None, :]
```

```python
import jax
import jax.numpy as jnp
from jax import lax
import jax.experimental.pallas as pl
import jax.experimental.pallas.tpu as pltpu

F32 = jnp.float32
BF16 = jnp.bfloat16

_STREAMS = 6
_CG = 32
_READ_SIZES = (64, 64, 64, 64, 64, 32, 16, 8, 4, 2, 1, 1)


def _se_kernel(x_hbm, wdt_ref, wu_ref, o_hbm, buf, scale_ref, in_sems, out_sem):
    A, HL, C, W = buf.shape
    n_lane = W // 128
    chunks = []
    pos = 0
    for sz in _READ_SIZES:
        a, r = divmod(pos, HL)
        assert r + sz <= HL
        chunks.append((a, r, sz))
        pos += sz
    assert pos == A * HL

    def rd(i):
        a, r, sz = chunks[i]
        idx = (a, pl.ds(r, sz))
        return pltpu.make_async_copy(x_hbm.at[idx], buf.at[idx], in_sems.at[i])

    for i in range(len(chunks)):
        rd(i).start()

    acc = jnp.zeros((C, 128), F32)
    for i, (a, r, sz) in enumerate(chunks):
        rd(i).wait()

        def body(h, acc, a=a):
            xf = buf[a, h].astype(F32)
            for k in range(n_lane):
                acc = acc + xf[:, k * 128:(k + 1) * 128]
            return acc

        acc = body(r, acc) if sz == 1 else lax.fori_loop(r, r + sz, body, acc)

    total = jnp.sum(acc, axis=1, keepdims=True)
    mean = (total * (1.0 / (A * HL * W))).astype(BF16)
    mean_b = jnp.broadcast_to(mean, (C, 128))
    hdn = jnp.dot(wdt_ref[...], mean_b, preferred_element_type=F32)
    hdn = hdn.astype(BF16).astype(F32)
    hdn = (hdn * jax.nn.sigmoid(hdn)).astype(BF16)
    z = lax.dot_general(wu_ref[...], hdn, (((0,), (0,)), ((), ())),
                        preferred_element_type=F32)
    z = z.astype(BF16).astype(F32)
    scale_ref[...] = jax.nn.sigmoid(z).astype(BF16).astype(F32)

    def wbody(h, carry):
        for g in range(C // _CG):
            rows = slice(g * _CG, (g + 1) * _CG)
            sg = jnp.concatenate([scale_ref[rows, :]] * n_lane, axis=1)
            for a in range(A):
                v = buf[a, h, rows, :].astype(F32)
                buf[a, h, rows, :] = (v * sg).astype(BF16)
            idx = (slice(None), h, pl.ds(g * _CG, _CG))
            pltpu.make_async_copy(buf.at[idx], o_hbm.at[idx], out_sem).start()
        return carry

    lax.fori_loop(0, HL, wbody, 0)
    pltpu.make_async_copy(buf, o_hbm, out_sem).wait()


@jax.jit
def pallas_standalone__se_block__vision_kernel(
    x: jax.Array,
    w_down: jax.Array,
    w_up: jax.Array,
):
    N, H, W, C = x.shape
    assert N == 1
    xt = jnp.transpose(x, (0, 1, 3, 2)).reshape(_STREAMS, H // _STREAMS, C, W)
    out = pl.pallas_call(
        _se_kernel,
        out_shape=jax.ShapeDtypeStruct(xt.shape, x.dtype),
        in_specs=[pl.BlockSpec(memory_space=pl.ANY),
                  pl.BlockSpec(memory_space=pltpu.VMEM),
                  pl.BlockSpec(memory_space=pltpu.VMEM)],
        out_specs=pl.BlockSpec(memory_space=pl.ANY),
        scratch_shapes=[pltpu.VMEM(xt.shape, x.dtype),
                        pltpu.VMEM((C, 128), F32),
                        pltpu.SemaphoreType.DMA((len(_READ_SIZES),)),
                        pltpu.SemaphoreType.DMA(())],
        compiler_params=pltpu.CompilerParams(vmem_limit_bytes=100 * 1024 * 1024),
    )(xt, w_down.T, w_up)
    return jnp.transpose(out.reshape(N, H, C, W), (0, 1, 3, 2))
```

```python
import jax
import jax.numpy as jnp
from jax import lax
import jax.experimental.pallas as pl
import jax.experimental.pallas.tpu as pltpu

F32 = jnp.float32
BF16 = jnp.bfloat16

_Q = 16
_G, _A = 6, 6
_MAIN = (8, 208, 108, 36)
_PART = (14, 6, 3, 1)
_FIN = (20, 4)


def _tree_sum(xs):
    xs = list(xs)
    while len(xs) > 1:
        nxt = [xs[i] + xs[i + 1] for i in range(0, len(xs) - 1, 2)]
        if len(xs) % 2:
            nxt.append(xs[-1])
        xs = nxt
    return xs[0]


def _se_kernel(x_hbm, wdt_hbm, wu_hbm, o_hbm,
               buf, wdt_v, wu_v, wub, wdf, scale, hp_ref, g_ref,
               in_sems, w_sems, out_sem):
    H, C, W = buf.shape
    R = wdt_v.shape[0]
    Q, G, A = _Q, _G, _A
    NL = W // 128
    NQ = C // Q
    CM = C - Q
    B = H * NQ // (G * A)
    bufs = buf.reshape(G, A, B, Q, W)

    chunks = []
    r = 0
    for n in _MAIN:
        chunks.append((r, n, 0, C))
        r += n
    r_split = r
    for n in _PART:
        chunks.append((r, n, 0, CM))
        r += n
    assert r == H
    r = r_split
    for n in _FIN:
        chunks.append((r, n, CM, Q))
        r += n
    assert r == H

    def rd(i):
        r0, n, c0, nc = chunks[i]
        idx = (pl.ds(r0, n), pl.ds(c0, nc))
        return pltpu.make_async_copy(x_hbm.at[idx], buf.at[idx], in_sems.at[i])

    wd_cp = pltpu.make_async_copy(wdt_hbm, wdt_v, w_sems.at[0])
    wu_cp = pltpu.make_async_copy(wu_hbm, wu_v, w_sems.at[1])

    rd(0).start(priority=1)
    wd_cp.start(priority=0)
    wu_cp.start(priority=0)
    for i in range(1, len(chunks)):
        rd(i).start(priority=1)

    wd_cp.wait()
    wu_cp.wait()
    row = lax.broadcasted_iota(jnp.int32, (R, 128), 0)
    for j in range(R):
        e = jnp.where(row == j, 1.0, 0.0).astype(BF16)
        wub[j] = lax.dot_general(wu_v[...], e, (((0,), (0,)), ((), ())),
                                 preferred_element_type=F32)
    wdt_f = wdt_v[...].astype(F32)
    for c in range(Q):
        wdf[c] = jnp.broadcast_to(wdt_f[:, CM + c:CM + c + 1], (R, 128))

    def add_row(h, accs, q0, q1):
        out = list(accs)
        for q in range(q0, q1):
            xf = buf[h, q * Q:(q + 1) * Q, :].astype(F32)
            out[q - q0] = out[q - q0] + _tree_sum(
                [xf[:, k * 128:(k + 1) * 128] for k in range(NL)])
        return tuple(out)

    def reduce_chunk(i, accs, q0, q1, unroll_all=False):
        r0, n, _, _ = chunks[i]
        if n == 1 or unroll_all:
            for h in range(r0, r0 + n):
                accs = add_row(h, accs, q0, q1)
            return accs
        return lax.fori_loop(r0, r0 + n, lambda h, a: add_row(h, a, q0, q1), accs)

    accs = tuple(jnp.zeros((Q, 128), F32) for _ in range(NQ))
    i = 0
    for _ in _MAIN:
        rd(i).wait()
        accs = reduce_chunk(i, accs, 0, NQ)
        i += 1
    acc_m, acc_f = accs[:-1], accs[-1:]
    for _ in _PART:
        rd(i).wait()
        acc_m = reduce_chunk(i, acc_m, 0, NQ - 1)
        i += 1

    inv = 1.0 / (H * W)
    tot_m = jnp.sum(jnp.concatenate(acc_m, axis=0), axis=1, keepdims=True)
    mean_m = jnp.broadcast_to((tot_m * inv).astype(BF16), (CM, 128))
    hp_ref[...] = jnp.dot(wdt_v[:, :CM], mean_m, preferred_element_type=F32)

    for k in range(len(_FIN)):
        rd(i).wait()
        r0, n, _, _ = chunks[i]
        if k == len(_FIN) - 1:
            parts = [acc_f[0]]
            for h in range(r0, r0 + n):
                xf = buf[h, CM:C, :].astype(F32)
                parts += [xf[:, kk * 128:(kk + 1) * 128] for kk in range(NL)]
            acc_f = (_tree_sum(parts),)
        else:
            acc_f = reduce_chunk(i, acc_f, NQ - 1, NQ, unroll_all=True)
        i += 1

    tot_f = jnp.sum(acc_f[0], axis=1, keepdims=True)
    mean_f = jnp.broadcast_to((tot_f * inv).astype(BF16).astype(F32), (Q, 128))
    hdn = _tree_sum(
        [hp_ref[...]]
        + [jnp.broadcast_to(mean_f[c:c + 1, :], (R, 128)) * wdf[c] for c in range(Q)])
    hdn = hdn.astype(BF16).astype(F32)
    g = (hdn * jax.nn.sigmoid(hdn)).astype(BF16).astype(F32)
    g_ref[...] = g

    def gate(g, q):
        if isinstance(q, int):
            rows = pl.ds(q * Q, Q)
        else:
            rows = pl.ds(pl.multiple_of(q * Q, Q), Q)
        z = _tree_sum([jnp.broadcast_to(g[j:j + 1, :], (Q, 128)) * wub[j, rows, :]
                       for j in range(R)])
        z = z.astype(BF16).astype(F32)
        return jax.nn.sigmoid(z).astype(BF16).astype(F32)

    offs = [(a * B) % NQ for a in range(A)]
    assert (A * B) % NQ == 0
    uoffs = sorted(set(offs))
    n_peel = NQ // len(uoffs)
    assert sorted((o + i) % NQ for o in uoffs for i in range(n_peel)) == list(range(NQ))
    assert max(uoffs) + n_peel <= NQ

    def scale_block(gi, a, i, s):
        s3 = jnp.concatenate([s] * NL, axis=1)
        v = bufs[gi, a, i].astype(F32)
        bufs[gi, a, i] = (v * s3).astype(BF16)

    def wr(gi, i):
        return pltpu.make_async_copy(bufs.at[gi, :, i], o_hbm.at[gi, :, i], out_sem)

    def peel(i, g):
        svals = {}
        for o in uoffs:
            svals[o] = gate(g, o + i)
            scale[o + i] = svals[o]
        for a in range(A):
            scale_block(0, a, i, svals[offs[a]])
        wr(0, i).start()

    peel(0, g)

    def pbody(i, carry):
        peel(i, g_ref[...])
        return carry

    lax.fori_loop(1, n_peel, pbody, 0)

    def wbody(t, carry):
        gi = t // B
        i = t % B
        q0 = i % NQ
        svals = {}
        for a in range(A):
            if offs[a] not in svals:
                q = q0 + offs[a]
                q = jnp.where(q >= NQ, q - NQ, q)
                svals[offs[a]] = scale[q]
            scale_block(gi, a, i, svals[offs[a]])
        wr(gi, i).start()
        return carry

    lax.fori_loop(n_peel, G * B, wbody, 0)
    pltpu.make_async_copy(bufs, o_hbm, out_sem).wait()


@jax.jit
def pallas_standalone__se_block__vision_kernel(
    x: jax.Array,
    w_down: jax.Array,
    w_up: jax.Array,
):
    N, H, W, C = x.shape
    R = w_down.shape[1]
    assert N == 1
    NQ = C // _Q
    B = H * NQ // (_G * _A)
    xt = jnp.transpose(x, (0, 1, 3, 2)).reshape(H, C, W)
    n_in = len(_MAIN) + len(_PART) + len(_FIN)
    out = pl.pallas_call(
        _se_kernel,
        out_shape=jax.ShapeDtypeStruct((_G, _A, B, _Q, W), x.dtype),
        in_specs=[pl.BlockSpec(memory_space=pl.ANY)] * 3,
        out_specs=pl.BlockSpec(memory_space=pl.ANY),
        scratch_shapes=[
            pltpu.VMEM((H, C, W), x.dtype),
            pltpu.VMEM((R, C), x.dtype),
            pltpu.VMEM((R, C), x.dtype),
            pltpu.VMEM((R, C, 128), F32),
            pltpu.VMEM((_Q, R, 128), F32),
            pltpu.VMEM((NQ, _Q, 128), F32),
            pltpu.VMEM((R, 128), F32),
            pltpu.VMEM((R, 128), F32),
            pltpu.SemaphoreType.DMA((n_in,)),
            pltpu.SemaphoreType.DMA((2,)),
            pltpu.SemaphoreType.DMA(()),
        ],
        compiler_params=pltpu.CompilerParams(
            vmem_limit_bytes=100 * 1024 * 1024,
            disable_bounds_checks=True,
            disable_semaphore_checks=True,
        ),
    )(xt, w_down.T, w_up)
    return jnp.transpose(out.reshape(N, H, C, W), (0, 1, 3, 2))
```

```python
import functools
import jax
import jax.numpy as jnp
from jax import lax
from jax.experimental import pallas as pl
from jax.experimental.pallas import tpu as pltpu

F32 = jnp.float32
BF16 = jnp.bfloat16


def _tree_sum(xs):
    xs = list(xs)
    while len(xs) > 1:
        nxt = [xs[i] + xs[i + 1] for i in range(0, len(xs) - 1, 2)]
        if len(xs) % 2:
            nxt.append(xs[-1])
        xs = nxt
    return xs[0]


def _sig(x, fast):
    if fast:
        return 0.5 * jnp.tanh(0.5 * x) + 0.5
    return jax.nn.sigmoid(x)


def build(main=(8, 208, 108, 36), part=(14, 6, 3, 1), fin=(20, 4), nf=3, A=6, B=64, PT=8, checks=False, fast=False):
    def kernel(x_hbm, wdt_hbm, wu_hbm, o_hbm, buf, wdt_v, wu_v, wub, wdf, stab, hp_ref, g_ref, in_sems, w_sems, out_sem):
        H, NV = buf.shape[0], buf.shape[1]
        R, C = wdt_v.shape
        NB = C // 8
        NT = 2 * NV
        NL = NT // NB
        W = NL * 128
        G = o_hbm.shape[0]
        NP = NT // PT
        assert NP * PT == NT
        bufs = buf.reshape(G, A, B, PT * 8, 128)
        VM = NV - nf
        BM = (2 * VM) // NL if (2 * VM) % NL == 0 else (2 * VM) // NL
        NFB = NB - BM

        chunks = []
        r = 0
        for n in main:
            chunks.append((r, n, 0, NV)); r += n
        r_split = r
        for n in part:
            chunks.append((r, n, 0, VM)); r += n
        assert r == H
        r = r_split
        for n in fin:
            chunks.append((r, n, VM, nf)); r += n
        assert r == H

        def rd(i):
            r0, n, v0, nv = chunks[i]
            idx = (pl.ds(r0, n), pl.ds(v0, nv))
            return pltpu.make_async_copy(x_hbm.at[idx], buf.at[idx], in_sems.at[i])

        wd_cp = pltpu.make_async_copy(wdt_hbm, wdt_v, w_sems.at[0])
        wu_cp = pltpu.make_async_copy(wu_hbm, wu_v, w_sems.at[1])
        rd(0).start(priority=1)
        wd_cp.start(priority=0)
        wu_cp.start(priority=0)
        for i in range(1, len(chunks)):
            rd(i).start(priority=1)

        wd_cp.wait()
        wu_cp.wait()
        row = lax.broadcasted_iota(jnp.int32, (R, 128), 0)
        for j in range(R):
            e = jnp.where(row == j, 1.0, 0.0).astype(BF16)
            wub[j] = lax.dot_general(wu_v[...], e, (((0,), (0,)), ((), ())), preferred_element_type=F32)
        wdt_f = wdt_v[...].astype(F32)
        for c in range(NFB * 8):
            wdf[c] = jnp.broadcast_to(wdt_f[:, BM * 8 + c:BM * 8 + c + 1], (R, 128))

        def row_tiles(h, v0, nv):
            d = {}
            for v in range(v0, v0 + nv):
                xf = buf[h, v].astype(F32)
                d.setdefault((2 * v) // NL, []).append(xf[:8])
                d.setdefault((2 * v + 1) // NL, []).append(xf[8:])
            return d

        def reduce_chunk(i, accs, unroll_all=False):
            r0, n, v0, nv = chunks[i]
            blocks = sorted({t // NL for t in range(2 * v0, 2 * (v0 + nv))})

            def body(h, sub):
                d = row_tiles(h, v0, nv)
                return tuple(s + _tree_sum(d[b]) for s, b in zip(sub, blocks))

            sub = tuple(accs[b] for b in blocks)
            if unroll_all == 'tree':
                ds = [row_tiles(h, v0, nv) for h in range(r0, r0 + n)]
                sub = tuple(_tree_sum([s] + [t for d in ds for t in d[b]]) for s, b in zip(sub, blocks))
            elif n == 1 or unroll_all:
                for h in range(r0, r0 + n):
                    sub = body(h, sub)
            else:
                sub = lax.fori_loop(r0, r0 + n, body, sub)
            accs = list(accs)
            for s, b in zip(sub, blocks):
                accs[b] = s
            return accs

        accs = [jnp.zeros((8, 128), F32) for _ in range(NB)]
        i = 0
        for _ in range(len(main) + len(part)):
            rd(i).wait()
            accs = reduce_chunk(i, accs)
            i += 1

        inv = 1.0 / (H * W)
        early = jnp.concatenate(accs[:BM] + [jnp.zeros((8, 128), F32)] * (BM % 2), axis=0)
        KM = early.shape[0]
        tot_m = jnp.sum(early, axis=1, keepdims=True)
        mean_m = jnp.broadcast_to((tot_m * inv).astype(BF16), (KM, 128))
        hp_ref[...] = jnp.dot(wdt_v[:, :KM], mean_m, preferred_element_type=F32)

        for k in range(len(fin)):
            rd(i).wait()
            accs = reduce_chunk(i, accs, unroll_all='tree' if k == len(fin) - 1 else True)
            i += 1

        terms = [hp_ref[...]]
        for b in range(BM, NB):
            tot = jnp.sum(accs[b], axis=1, keepdims=True)
            m = jnp.broadcast_to((tot * inv).astype(BF16).astype(F32), (8, 128))
            terms += [jnp.broadcast_to(m[c:c + 1, :], (R, 128)) * wdf[(b - BM) * 8 + c] for c in range(8)]
        hdn = _tree_sum(terms).astype(BF16).astype(F32)
        g = (hdn * _sig(hdn, fast)).astype(BF16).astype(F32)

        GB = 3
        assert NB % GB == 0 and GB * NL >= PT and NB // GB <= NP

        def gates(g, k):
            if isinstance(k, int):
                rows = pl.ds(k * GB * 8, GB * 8)
            else:
                rows = pl.ds(pl.multiple_of(k * (GB * 8), 8), GB * 8)
            z = _tree_sum([jnp.broadcast_to(g[j:j + 1, :], (GB * 8, 128)) * wub[j, rows, :] for j in range(R)])
            z = z.astype(BF16).astype(F32)
            s = _sig(z, fast).astype(BF16).astype(F32)
            tiles = [s[b * 8:(b + 1) * 8] for b in range(GB) for _ in range(NL)]
            return jnp.concatenate(tiles, axis=0)

        def put_gates(k, full):
            n = GB * NL * 8
            if isinstance(k, int):
                stab[pl.ds(k * n, n), :] = full
            else:
                stab[pl.ds(pl.multiple_of(k * n, 8), n), :] = full

        def scale_piece(gi, a, i, s):
            v = bufs[gi, a, i].astype(F32)
            bufs[gi, a, i] = (v * s).astype(BF16)

        def phase_scale(p):
            return stab[pl.ds(pl.multiple_of(p * (PT * 8), 8), PT * 8), :]

        sa = B % NP
        sg = (A * B) % NP
        assert sa == 1

        full0 = gates(g, 0)
        s0 = full0[:PT * 8]
        for a in range(A):
            i = (0 - a) % NP
            scale_piece(0, a, i, s0)
            pltpu.make_async_copy(bufs.at[0, a, i], o_hbm.at[0, a, i], out_sem).start()
        put_gates(0, full0)
        g_ref[...] = g

        def pbody(p, carry):
            k = jnp.minimum(p, NB // GB - 1)
            idx = [jnp.where(p >= a, p - a, p - a + NP) for a in range(A)]
            vals = [bufs[0, a, idx[a]] for a in range(A)]
            put_gates(k, gates(g_ref[...], k))
            s = phase_scale(p)
            for a in range(A):
                bufs[0, a, idx[a]] = (vals[a].astype(F32) * s).astype(BF16)
            for a in range(A):
                pltpu.make_async_copy(bufs.at[0, a, idx[a]], o_hbm.at[0, a, idx[a]], out_sem).start()
            return carry

        lax.fori_loop(1, NP, pbody, 0)

        def wbody(t, carry):
            gi = t // B
            i = t % B
            p0 = (gi * sg + i) % NP
            for a in range(A):
                p = p0 + a
                p = jnp.where(p >= NP, p - NP, p)
                scale_piece(gi, a, i, phase_scale(p))
            pltpu.make_async_copy(bufs.at[gi, :, i], o_hbm.at[gi, :, i], out_sem).start()
            return carry

        lax.fori_loop(NP, G * B, wbody, 0)
        pltpu.make_async_copy(bufs, o_hbm, out_sem).wait()

    def se_fn(x, w_down, w_up):
        N, H, W, C = x.shape
        R = w_down.shape[1]
        assert N == 1
        NB, NL = C // 8, W // 128
        NV = NB * NL // 2
        G = H * NB * NL // (A * B * PT)
        xt = x.reshape(H, NL, 128, NB, 8).transpose(0, 3, 1, 4, 2).reshape(H, NV, 16, 128)
        n_in = len(main) + len(part) + len(fin)
        nfb = NB - (2 * (NV - nf)) // NL
        out = pl.pallas_call(
            kernel,
            out_shape=jax.ShapeDtypeStruct((G, A, B, PT * 8, 128), x.dtype),
            in_specs=[pl.BlockSpec(memory_space=pl.ANY)] * 3,
            out_specs=pl.BlockSpec(memory_space=pl.ANY),
            scratch_shapes=[pltpu.VMEM((H, NV, 16, 128), x.dtype),
                            pltpu.VMEM((R, C), x.dtype),
                            pltpu.VMEM((R, C), x.dtype),
                            pltpu.VMEM((R, C, 128), F32),
                            pltpu.VMEM((nfb * 8, R, 128), F32),
                            pltpu.VMEM((NB * NL * 8, 128), F32),
                            pltpu.VMEM((R, 128), F32),
                            pltpu.VMEM((R, 128), F32),
                            pltpu.SemaphoreType.DMA((n_in,)),
                            pltpu.SemaphoreType.DMA((2,)),
                            pltpu.SemaphoreType.DMA(())],
            compiler_params=pltpu.CompilerParams(
                vmem_limit_bytes=100 * 1024 * 1024,
                disable_bounds_checks=not checks,
                disable_semaphore_checks=not checks),
        )(xt, w_down.T, w_up)
        out = out.reshape(H, NB, NL, 8, 128).transpose(0, 2, 4, 1, 3).reshape(N, H, W, C)
        return out
    return se_fn


_impl = build(**dict())


@jax.jit
def pallas_standalone__se_block__vision_kernel(x: jax.Array, w_down: jax.Array, w_up: jax.Array):
    return _impl(x, w_down, w_up)
```

```python
import jax
import jax.numpy as jnp
from jax import lax
import jax.experimental.pallas as pl
import jax.experimental.pallas.tpu as pltpu

F32 = jnp.float32
BF16 = jnp.bfloat16

_MAIN = (8, 208, 108, 36)
_PART = (14, 6, 3, 1)
_FIN = (20, 4)
_LATE = 3
_STREAMS = 6
_STREAM_LEN = 64
_PIECE = 4
_RING = 8
_GATE_BLOCKS = 3


def _tree_sum(xs):
    xs = list(xs)
    while len(xs) > 1:
        nxt = [xs[i] + xs[i + 1] for i in range(0, len(xs) - 1, 2)]
        if len(xs) % 2:
            nxt.append(xs[-1])
        xs = nxt
    return xs[0]


def _round_bf16(x):
    return x.astype(BF16).astype(F32)


def _sigmoid_bf16(x):
    d = _round_bf16(1.0 + _round_bf16(jnp.exp(-x)))
    return _round_bf16(pl.reciprocal(d, approx=True))


def _se_kernel(x_hbm, wdt_hbm, wu_hbm, o_hbm,
               buf, wdt_v, wu_v, wub, wdf, stab, hp_ref, g_ref,
               in_sems, w_sems, out_sems):
    H, NV = buf.shape[0], buf.shape[1]
    R, C = wdt_v.shape
    A, B, PV, D, GB = _STREAMS, _STREAM_LEN, _PIECE, _RING, _GATE_BLOCKS
    NB = C // 8
    NL = 2 * NV // NB
    W = NL * 128
    NP = NV // PV
    T = H * NP // A
    VM = NV - _LATE
    BM = (2 * VM) // NL
    PR = PV * 16
    SH, SA = divmod(B, NP)
    assert NP * PV == NV and (H * NP) % (A * B) == 0 and BM % 2 == 0
    assert NB % GB == 0 and GB * NL >= 2 * PV and NB // GB <= NP
    assert SA == 1 and A <= NP and T - NP >= D

    chunks = []
    r = 0
    for n in _MAIN:
        chunks.append((r, n, 0, NV))
        r += n
    r_split = r
    for n in _PART:
        chunks.append((r, n, 0, VM))
        r += n
    assert r == H
    r = r_split
    for n in _FIN:
        chunks.append((r, n, VM, _LATE))
        r += n
    assert r == H

    def rd(i):
        r0, n, v0, nv = chunks[i]
        idx = (pl.ds(r0, n), pl.ds(v0, nv))
        return pltpu.make_async_copy(x_hbm.at[idx], buf.at[idx], in_sems.at[i])

    wd_cp = pltpu.make_async_copy(wdt_hbm, wdt_v, w_sems.at[0])
    wu_cp = pltpu.make_async_copy(wu_hbm, wu_v, w_sems.at[1])
    rd(0).start(priority=1)
    wd_cp.start(priority=0)
    wu_cp.start(priority=0)
    for i in range(1, len(chunks)):
        rd(i).start(priority=1)

    wd_cp.wait()
    wu_cp.wait()
    row = lax.broadcasted_iota(jnp.int32, (R, 128), 0)
    for j in range(R):
        pick = jnp.where(row == j, 1.0, 0.0).astype(BF16)
        wub[j] = lax.dot_general(wu_v[...], pick, (((0,), (0,)), ((), ())),
                                 preferred_element_type=F32)
    wdt_f = wdt_v[...].astype(F32)
    for c in range((NB - BM) * 8):
        wdf[c] = jnp.broadcast_to(wdt_f[:, BM * 8 + c:BM * 8 + c + 1], (R, 128))

    def row_tiles(h, v0, nv):
        tiles = {}
        for v in range(v0, v0 + nv):
            xf = buf[h, v].astype(F32)
            tiles.setdefault((2 * v) // NL, []).append(xf[:8])
            tiles.setdefault((2 * v + 1) // NL, []).append(xf[8:])
        return tiles

    def reduce_chunk(i, accs, mode):
        r0, n, v0, nv = chunks[i]
        blocks = sorted({t // NL for t in range(2 * v0, 2 * (v0 + nv))})

        def body(h, sub):
            tiles = row_tiles(h, v0, nv)
            return tuple(s + _tree_sum(tiles[b]) for s, b in zip(sub, blocks))

        sub = tuple(accs[b] for b in blocks)
        if mode == "tree":
            rows = [row_tiles(h, v0, nv) for h in range(r0, r0 + n)]
            sub = tuple(_tree_sum([s] + [t for tiles in rows for t in tiles[b]])
                        for s, b in zip(sub, blocks))
        elif mode == "unroll" or n == 1:
            for h in range(r0, r0 + n):
                sub = body(h, sub)
        else:
            sub = lax.fori_loop(r0, r0 + n, body, sub)
        accs = list(accs)
        for s, b in zip(sub, blocks):
            accs[b] = s
        return accs

    n_early = len(_MAIN) + len(_PART)
    accs = [jnp.zeros((8, 128), F32) for _ in range(NB)]
    for i in range(n_early):
        rd(i).wait()
        accs = reduce_chunk(i, accs, "loop")

    inv = 1.0 / (H * W)
    tot_m = jnp.sum(jnp.concatenate(accs[:BM], axis=0), axis=1, keepdims=True)
    mean_m = jnp.broadcast_to((tot_m * inv).astype(BF16), (BM * 8, 128))
    hp_ref[...] = jnp.dot(wdt_v[:, :BM * 8], mean_m, preferred_element_type=F32)

    for i in range(n_early, len(chunks)):
        rd(i).wait()
        accs = reduce_chunk(i, accs, "tree" if i == len(chunks) - 1 else "unroll")

    terms = [hp_ref[...]]
    for b in range(BM, NB):
        tot = jnp.sum(accs[b], axis=1, keepdims=True)
        m = jnp.broadcast_to(_round_bf16(tot * inv), (8, 128))
        terms += [jnp.broadcast_to(m[c:c + 1, :], (R, 128)) * wdf[(b - BM) * 8 + c]
                  for c in range(8)]
    hdn = _round_bf16(_tree_sum(terms))
    g = _round_bf16(hdn * _sigmoid_bf16(hdn))

    def aligned(k, n):
        return k * n if isinstance(k, int) else pl.multiple_of(k * n, 8)

    def gates(g, k):
        rows = pl.ds(aligned(k, GB * 8), GB * 8)
        z = _tree_sum([jnp.broadcast_to(g[j:j + 1, :], (GB * 8, 128)) * wub[j, rows, :]
                       for j in range(R)])
        s = _sigmoid_bf16(_round_bf16(z))
        return jnp.concatenate(
            [s[b * 8:(b + 1) * 8] for b in range(GB) for _ in range(NL)], axis=0)

    def put_gates(k, full):
        stab[pl.ds(aligned(k, GB * NL * 8), GB * NL * 8), :] = full

    def piece_gate(p):
        return stab[pl.ds(aligned(p, PR), PR), :].reshape(PV, 16, 128)

    def scaled(v, s):
        return (v.astype(F32) * s).astype(BF16)

    def wr(h, p, sem):
        idx = (h, pl.ds(p * PV, PV))
        return pltpu.make_async_copy(buf.at[idx], o_hbm.at[idx], sem)

    head_sem = out_sems.at[D]
    full0 = gates(g, 0)
    s0 = full0[:PR].reshape(PV, 16, 128)
    for a in range(A):
        h = SH * a + (1 if a > 0 else 0)
        buf[h, 0:PV] = scaled(buf[h, 0:PV], s0)
        wr(h, 0, head_sem).start()
    g_ref[...] = g

    def head_rows(p):
        return [SH * a + jnp.where(p >= a, 0, 1) for a in range(A)]

    def head_step(p, carry):
        @pl.when(p == 1)
        def _():
            put_gates(0, full0)

        k = jnp.minimum(p, NB // GB - 1)
        hs = head_rows(p)
        cols = pl.ds(p * PV, PV)
        vals = [buf[h, cols] for h in hs]
        put_gates(k, gates(g_ref[...], k))
        s = piece_gate(p)
        for h, v in zip(hs, vals):
            buf[h, cols] = scaled(v, s)
        for h in hs:
            wr(h, p, head_sem).start()
        return carry

    lax.fori_loop(1, NP, head_step, 0)

    def pieces(t):
        if isinstance(t, int):
            first = (t // B) * (A * B) + t % B
            return [divmod(first + a * B, NP) for a in range(A)]
        first = lax.div(t, B) * (A * B) + lax.rem(t, B)
        h0, p0 = lax.div(first, NP), lax.rem(first, NP)
        out = []
        for a in range(A):
            wrap = p0 + a >= NP
            out.append((h0 + SH * a + jnp.where(wrap, 1, 0),
                        jnp.where(wrap, p0 + a - NP, p0 + a)))
        return out

    def step_sem(t):
        return out_sems.at[t % D if isinstance(t, int) else lax.rem(t, D)]

    def wait_step(t):
        for h, p in pieces(t):
            wr(h, p, step_sem(t)).wait()

    def step(t, carry):
        hp = pieces(t)
        vals = [buf[h, pl.ds(p * PV, PV)] for h, p in hp]
        for (h, p), v in zip(hp, vals):
            buf[h, pl.ds(p * PV, PV)] = scaled(v, piece_gate(p))

        @pl.when(t >= NP + D)
        def _():
            wait_step(t - D)

        for h, p in hp:
            wr(h, p, step_sem(t)).start()
        return carry

    lax.fori_loop(NP, T, step, 0)

    def drain_head(p, carry):
        for h in head_rows(p):
            wr(h, p, head_sem).wait()
        return carry

    lax.fori_loop(0, NP, drain_head, 0)
    for t in range(T - D, T):
        wait_step(t)


@jax.jit
def pallas_standalone__se_block__vision_kernel(
    x: jax.Array,
    w_down: jax.Array,
    w_up: jax.Array,
):
    N, H, W, C = x.shape
    R = w_down.shape[1]
    assert N == 1
    NB, NL = C // 8, W // 128
    NV = NB * NL // 2
    late_blocks = NB - (2 * (NV - _LATE)) // NL
    xt = x.reshape(H, NL, 128, NB, 8).transpose(0, 3, 1, 4, 2).reshape(H, NV, 16, 128)
    out = pl.pallas_call(
        _se_kernel,
        out_shape=jax.ShapeDtypeStruct(xt.shape, x.dtype),
        in_specs=[pl.BlockSpec(memory_space=pl.ANY)] * 3,
        out_specs=pl.BlockSpec(memory_space=pl.ANY),
        scratch_shapes=[
            pltpu.VMEM(xt.shape, x.dtype),
            pltpu.VMEM((R, C), w_down.dtype),
            pltpu.VMEM((R, C), w_up.dtype),
            pltpu.VMEM((R, C, 128), F32),
            pltpu.VMEM((late_blocks * 8, R, 128), F32),
            pltpu.VMEM((NB * NL * 8, 128), F32),
            pltpu.VMEM((R, 128), F32),
            pltpu.VMEM((R, 128), F32),
            pltpu.SemaphoreType.DMA((len(_MAIN) + len(_PART) + len(_FIN),)),
            pltpu.SemaphoreType.DMA((2,)),
            pltpu.SemaphoreType.DMA((_RING + 1,)),
        ],
        compiler_params=pltpu.CompilerParams(
            vmem_limit_bytes=100 * 1024 * 1024,
            disable_bounds_checks=True,
            disable_semaphore_checks=True,
        ),
    )(xt, w_down.T, w_up)
    return out.reshape(H, NB, NL, 8, 128).transpose(0, 2, 4, 1, 3).reshape(N, H, W, C)
```
